```python
import os as _os
_os.environ.setdefault("JAX_PLATFORMS", "cpu")
import jax
import jax.numpy as jnp

def _softmax(x, axis=-1):
    return jax.nn.softmax(x, axis=axis)
def _gelu(x):
    return jax.nn.gelu(x, approximate=True)
def _silu(x):
    return jax.nn.silu(x)
def _sigmoid(x):
    return jax.nn.sigmoid(x)
def _layernorm(x, axis=-1, eps=1e-5):
    m = jnp.mean(x, axis=axis, keepdims=True)
    v = jnp.var(x, axis=axis, keepdims=True)
    return (x - m) / jnp.sqrt(v + eps)
def _scatter_add(tgt, idx, src, axis=0):
    return tgt.at[idx].add(src)
def _segment_sum(src, seg, n):
    return jax.ops.segment_sum(src, seg, n)
class _Rng:
    def __init__(self, key):
        self._k = key
    def _next(self):
        self._k, sub = jax.random.split(self._k)
        return sub
    def normal(self, shape):
        return jax.random.normal(self._next(), shape, dtype=jnp.bfloat16)
    def randint(self, lo, hi, shape):
        return jax.random.randint(self._next(), shape, lo, hi, dtype=jnp.int32)
    def uniform(self, shape, lo=0.0, hi=1.0):
        return jax.random.uniform(self._next(), shape, jnp.bfloat16, lo, hi)
    def permutation(self, n):
        return jax.random.permutation(self._next(), n)


kernel_name = 'sequential_preLN__sliding_local_dilated__dense_activation_mish__prompt'

def setup_inputs():
    _rng = _Rng(jax.random.key(int.from_bytes(__import__("os").urandom(4), "little")))
    _w = (lambda a: (lambda t: t.astype(jnp.bfloat16) if jnp.issubdtype(t.dtype, jnp.floating) else t)(jnp.asarray(a)))
    def _A_setup():
        B, S, D = 1, 2048, 512
        return {
            "x": _w((lambda *s: _rng.normal(s) * 0.05)(B, S, D)),
            "wqkv": _w((lambda *s: _rng.normal(s) * 0.05)(D, 3 * D)),
            "wo": _w((lambda *s: _rng.normal(s) * 0.05)(D, D)),
        }
    _A_in = _A_setup()

    def _B_setup():
        B, S, D, F = 1, 2048, 512, 1376
        return {
            "x": _w((lambda *s: _rng.normal(s) * 0.05)(B, S, D)),
            "w1": _w((lambda *s: _rng.normal(s) * 1.6)(D, F) * (D ** -0.5)),
            "b1": _w((lambda *s: _rng.normal(s) * 0.1)(F)),
            "w2": _w((lambda *s: _rng.normal(s) * 0.1)(F, D) * (F ** -0.5)),
        }
    _B_in = _B_setup()

    return {
        "A_x": _A_in["x"],
        "A_wqkv": _A_in["wqkv"],
        "A_wo": _A_in["wo"],
        "B_x": _B_in["x"],
        "B_w1": _B_in["w1"],
        "B_b1": _B_in["b1"],
        "B_w2": _B_in["w2"],
    }

def reference(A_x, A_wqkv, A_wo, B_x, B_w1, B_b1, B_w2):
    def _A_ref(x, wqkv, wo):
        B, S, D = x.shape
        H = 32; Dh = D // H
        W, dil = 8, 2
        qkv = (lambda x, *d: x.transpose(*d))((x @ wqkv).reshape(B, S, 3, H, Dh), 2, 0, 3, 1, 4)
        q, k, v = qkv[0], qkv[1], qkv[2]
        scale = Dh ** -0.5
        pos = jnp.arange(S)
        off = jnp.arange(W) * dil
        idx = pos[:, None] - off[None, :]
        mask = idx >= 0
        idx_c = jnp.where(mask, idx, 0).reshape(-1)
        kg = k[:, :, idx_c, :].reshape(B, H, S, W, Dh)
        vg = v[:, :, idx_c, :].reshape(B, H, S, W, Dh)
        logits = jnp.einsum("bhsd,bhswd->bhsw", q, kg) * scale
        logits = jnp.where(mask[None, None, :, :], logits, -1e9)
        attn = _softmax(logits, axis=-1)
        o = jnp.einsum("bhsw,bhswd->bhsd", attn, vg)
        return (lambda x, *d: x.transpose(*d))(o, 0, 2, 1, 3).reshape(B, S, D) @ wo

    def _B_ref(x, w1, b1, w2):
        h = jnp.einsum("bsd,df->bsf", x, w1) + b1
        sp = jnp.log1p(jnp.exp(-jnp.abs(h))) + jnp.where(h > 0, h, jnp.zeros_like(h))
        act = h * jnp.tanh(sp)
        return jnp.einsum("bsf,fd->bsd", act, w2)

    x = A_x
    h = x + _A_ref(_layernorm(x, axis=-1), A_wqkv, A_wo)
    h2 = h + _B_ref(_layernorm(h, axis=-1), B_w1, B_b1, B_w2)
    return h2
```

```python
import functools

import jax
import jax.numpy as jnp
import jax.experimental.pallas as pl
import jax.experimental.pallas.tpu as pltpu

_H = 32
_DH = 16
_W = 8
_DIL = 2
_HALO = 16
_EPS = 1e-5


def _layernorm(x):
    m = jnp.mean(x, axis=-1, keepdims=True)
    xc = x - m
    v = jnp.mean(xc * xc, axis=-1, keepdims=True)
    return xc * jax.lax.rsqrt(v + _EPS)


def _mish(h):
    sp = jnp.log1p(jnp.exp(-jnp.abs(h))) + jnp.maximum(h, 0.0)
    return h * jnp.tanh(sp)


def _kernel(x_ref, wqkv_ref, wo_ref, w1_ref, b1_ref, w2_ref, o_ref,
            wqkv_p, wo_p, kbuf, vbuf, *, ts, d):
    i = pl.program_id(0)
    f32 = jnp.float32
    bf16 = jnp.bfloat16

    @pl.when(i == 0)
    def _():
        r = jax.lax.broadcasted_iota(jnp.int32, (d, d), 0)
        c = jax.lax.broadcasted_iota(jnp.int32, (d, d), 1)
        perm = (r == (c % _H) * _DH + c // _H)
        p1 = jnp.where(perm, 1.0, 0.0).astype(bf16)
        pq = jnp.where(perm, _DH ** -0.5, 0.0).astype(bf16)
        permt = (c == (r % _H) * _DH + r // _H)
        pt = jnp.where(permt, 1.0, 0.0).astype(bf16)
        wqkv_p[:, 0:d] = jnp.dot(wqkv_ref[:, 0:d], pq,
                                 preferred_element_type=f32).astype(bf16)
        wqkv_p[:, d:2 * d] = jnp.dot(wqkv_ref[:, d:2 * d], p1,
                                     preferred_element_type=f32).astype(bf16)
        wqkv_p[:, 2 * d:3 * d] = jnp.dot(wqkv_ref[:, 2 * d:3 * d], p1,
                                         preferred_element_type=f32).astype(bf16)
        wo_p[...] = jnp.dot(pt, wo_ref[...],
                            preferred_element_type=f32).astype(bf16)
        kbuf[0:_HALO, :] = jnp.zeros((_HALO, d), f32)
        vbuf[0:_HALO, :] = jnp.zeros((_HALO, d), f32)

    x = x_ref[...].astype(f32)
    ln1 = _layernorm(x).astype(bf16)
    qkv = jnp.dot(ln1, wqkv_p[...], preferred_element_type=f32)
    q = qkv[:, 0:d]
    kbuf[_HALO:_HALO + ts, :] = qkv[:, d:2 * d]
    vbuf[_HALO:_HALO + ts, :] = qkv[:, 2 * d:3 * d]

    pos = i * ts + jax.lax.broadcasted_iota(jnp.int32, (ts, 128), 0)
    logits = []
    for w in range(_W):
        kw = kbuf[pl.ds(_HALO - _DIL * w, ts), :]
        p = q * kw
        t = (p[:, 0:128] + p[:, 128:256]) + (p[:, 256:384] + p[:, 384:512])
        t = t + pltpu.roll(t, 32, 1)
        t = t + pltpu.roll(t, 64, 1)
        logits.append(jnp.where(pos >= _DIL * w, t, -1e9))
    m = logits[0]
    for w in range(1, _W):
        m = jnp.maximum(m, logits[w])
    es = [jnp.exp(l - m) for l in logits]
    den = es[0]
    for w in range(1, _W):
        den = den + es[w]
    inv = 1.0 / den
    accs = [None] * 4
    for w in range(_W):
        vw = vbuf[pl.ds(_HALO - _DIL * w, ts), :]
        for cidx in range(4):
            term = es[w] * vw[:, cidx * 128:(cidx + 1) * 128]
            accs[cidx] = term if accs[cidx] is None else accs[cidx] + term
    o = jnp.concatenate([a * inv for a in accs], axis=1).astype(bf16)

    kbuf[0:_HALO, :] = kbuf[ts:ts + _HALO, :]
    vbuf[0:_HALO, :] = vbuf[ts:ts + _HALO, :]

    h = x + jnp.dot(o, wo_p[...], preferred_element_type=f32)
    ln2 = _layernorm(h).astype(bf16)
    h1 = jnp.dot(ln2, w1_ref[...], preferred_element_type=f32)
    h1 = h1 + b1_ref[...].astype(f32)
    act = _mish(h1).astype(bf16)
    out = h + jnp.dot(act, w2_ref[...], preferred_element_type=f32)
    o_ref[...] = out.astype(o_ref.dtype)


@jax.jit
def pallas_sequential_preLN__sliding_local_dilated__dense_activation_mish__prompt_kernel(
    A_x: jax.Array,
    A_wqkv: jax.Array,
    A_wo: jax.Array,
    B_x: jax.Array,
    B_w1: jax.Array,
    B_b1: jax.Array,
    B_w2: jax.Array,
):
    B, S, D = A_x.shape
    F = B_w1.shape[1]
    assert B == 1 and D == _H * _DH
    ts = 256
    x2 = A_x.reshape(S, D)
    b1 = B_b1.reshape(1, F)

    kernel = functools.partial(_kernel, ts=ts, d=D)
    out = pl.pallas_call(
        kernel,
        grid=(S // ts,),
        in_specs=[
            pl.BlockSpec((ts, D), lambda i: (i, 0)),
            pl.BlockSpec((D, 3 * D), lambda i: (0, 0)),
            pl.BlockSpec((D, D), lambda i: (0, 0)),
            pl.BlockSpec((D, F), lambda i: (0, 0)),
            pl.BlockSpec((1, F), lambda i: (0, 0)),
            pl.BlockSpec((F, D), lambda i: (0, 0)),
        ],
        out_specs=pl.BlockSpec((ts, D), lambda i: (i, 0)),
        out_shape=jax.ShapeDtypeStruct((S, D), A_x.dtype),
        scratch_shapes=[
            pltpu.VMEM((D, 3 * D), jnp.bfloat16),
            pltpu.VMEM((D, D), jnp.bfloat16),
            pltpu.VMEM((ts + _HALO, D), jnp.float32),
            pltpu.VMEM((ts + _HALO, D), jnp.float32),
        ],
        compiler_params=pltpu.CompilerParams(
            dimension_semantics=("arbitrary",),
            vmem_limit_bytes=100 * 1024 * 1024,
        ),
    )(x2, A_wqkv, A_wo, B_w1, b1, B_w2)
    return out.reshape(B, S, D)
```

```python
import functools

import jax
import jax.numpy as jnp
import jax.experimental.pallas as pl
import jax.experimental.pallas.tpu as pltpu

_H = 32
_DH = 16
_W = 8
_DIL = 2
_HALO = 16
_EPS = 1e-5


def _layernorm(x):
    m = jnp.mean(x, axis=-1, keepdims=True)
    xc = x - m
    v = jnp.mean(xc * xc, axis=-1, keepdims=True)
    return xc * jax.lax.rsqrt(v + _EPS)


def _mish(h):
    sp = jnp.log1p(jnp.exp(-jnp.abs(h))) + jnp.maximum(h, 0.0)
    return h * jnp.tanh(sp)


def _dot_t(a, b):
    return jax.lax.dot_general(a, b, (((1,), (1,)), ((), ())),
                               preferred_element_type=jnp.float32)


def _kernel(x_ref, b1_ref, wqkv_raw, wo_raw, w1_hbm, w2_hbm, o_ref,
            w1_v, w2_v, wqkv_p, wo_p, tmp, kbuf, vbuf, sems,
            *, ts, sub, d):
    i = pl.program_id(0)
    f32 = jnp.float32
    bf16 = jnp.bfloat16

    def prologue():
        cps = [
            pltpu.make_async_copy(w1_hbm, w1_v, sems.at[0]),
            pltpu.make_async_copy(w2_hbm, w2_v, sems.at[1]),
        ]
        for cp in cps:
            cp.start()
        kbuf[0:_HALO, :] = jnp.zeros((_HALO, d), f32)
        vbuf[0:_HALO, :] = jnp.zeros((_HALO, d), f32)

        def permute_rows(dst, base):
            for c in range(d // 128):
                for dd in range(_DH):
                    dst[base + dd * _H:base + (dd + 1) * _H, c * 128:(c + 1) * 128] = (
                        tmp[c, pl.ds(dd, _H, stride=_DH), :].astype(bf16))

        for part in range(3):
            wt = wqkv_raw[:, part * d:(part + 1) * d].astype(f32).T
            for c in range(d // 128):
                tmp[c] = wt[:, c * 128:(c + 1) * 128]
            permute_rows(wqkv_p, part * d)
        wt = wo_raw[...].astype(f32)
        for c in range(d // 128):
            tmp[c] = wt[:, c * 128:(c + 1) * 128]
        permute_rows(wo_p, 0)
        return cps

    nsub = ts // sub

    def stage_qkv(j):
        r0 = j * sub
        x = x_ref[r0:r0 + sub, :].astype(f32)
        ln1 = _layernorm(x).astype(bf16)
        qkv = _dot_t(ln1, wqkv_p[...])
        kbuf[_HALO + r0:_HALO + r0 + sub, :] = qkv[:, d:2 * d]
        vbuf[_HALO + r0:_HALO + r0 + sub, :] = qkv[:, 2 * d:3 * d]
        return x, qkv[:, 0:d]

    def stage_attn(j, q):
        r0 = j * sub
        pos = i * ts + r0 + jax.lax.broadcasted_iota(jnp.int32, (sub, 128), 0)
        logits = []
        for w in range(_W):
            kw = kbuf[pl.ds(_HALO + r0 - _DIL * w, sub), :]
            p = q * kw
            t = (p[:, 0:128] + p[:, 128:256]) + (p[:, 256:384] + p[:, 384:512])
            t = t + pltpu.roll(t, 32, 1)
            t = (t + pltpu.roll(t, 64, 1)) * (_DH ** -0.5)
            logits.append(jnp.where(pos >= _DIL * w, t, -1e9))
        m = logits[0]
        for w in range(1, _W):
            m = jnp.maximum(m, logits[w])
        es = [jnp.exp(l - m) for l in logits]
        den = es[0]
        for w in range(1, _W):
            den = den + es[w]
        inv = 1.0 / den
        accs = [None] * 4
        for w in range(_W):
            vw = vbuf[pl.ds(_HALO + r0 - _DIL * w, sub), :]
            for cidx in range(4):
                term = es[w] * vw[:, cidx * 128:(cidx + 1) * 128]
                accs[cidx] = term if accs[cidx] is None else accs[cidx] + term
        return jnp.concatenate([a * inv for a in accs], axis=1).astype(bf16)

    def stage_mlp(j, x, o):
        r0 = j * sub
        h = x + jnp.dot(o, wo_p[...], preferred_element_type=f32)
        ln2 = _layernorm(h).astype(bf16)
        h1 = _dot_t(ln2, w1_v[...])
        h1 = h1 + b1_ref[...].astype(f32)
        act = _mish(h1).astype(bf16)
        out = h + jnp.dot(act, w2_v[...], preferred_element_type=f32)
        o_ref[r0:r0 + sub, :] = out.astype(o_ref.dtype)

    def body(first):
        if first:
            cps = prologue()
        xs, qs = [], []
        for j in range(nsub):
            x, q = stage_qkv(j)
            xs.append(x)
            qs.append(q)
        for j in range(nsub):
            o = stage_attn(j, qs[j])
            if first and j == 0:
                cps[0].wait()
                cps[1].wait()
            stage_mlp(j, xs[j], o)

    pl.when(i == 0)(lambda: body(True))
    pl.when(i > 0)(lambda: body(False))

    kbuf[0:_HALO, :] = kbuf[ts:ts + _HALO, :]
    vbuf[0:_HALO, :] = vbuf[ts:ts + _HALO, :]


@jax.jit
def pallas_sequential_preLN__sliding_local_dilated__dense_activation_mish__prompt_kernel(
    A_x: jax.Array,
    A_wqkv: jax.Array,
    A_wo: jax.Array,
    B_x: jax.Array,
    B_w1: jax.Array,
    B_b1: jax.Array,
    B_w2: jax.Array,
):
    B, S, D = A_x.shape
    F = B_w1.shape[1]
    assert B == 1 and D == _H * _DH
    ts = 512
    sub = 256
    x2 = A_x.reshape(S, D)
    b1 = B_b1.reshape(1, F)
    bf16 = jnp.bfloat16

    kernel = functools.partial(_kernel, ts=ts, sub=sub, d=D)
    out = pl.pallas_call(
        kernel,
        grid=(S // ts,),
        in_specs=[
            pl.BlockSpec((ts, D), lambda i: (i, 0)),
            pl.BlockSpec((1, F), lambda i: (0, 0)),
            pl.BlockSpec((D, 3 * D), lambda i: (0, 0)),
            pl.BlockSpec((D, D), lambda i: (0, 0)),
            pl.BlockSpec(memory_space=pl.ANY),
            pl.BlockSpec(memory_space=pl.ANY),
        ],
        out_specs=pl.BlockSpec((ts, D), lambda i: (i, 0)),
        out_shape=jax.ShapeDtypeStruct((S, D), A_x.dtype),
        scratch_shapes=[
            pltpu.VMEM((F, D), bf16),
            pltpu.VMEM((F, D), bf16),
            pltpu.VMEM((3 * D, D), bf16),
            pltpu.VMEM((D, D), bf16),
            pltpu.VMEM((D // 128, D, 128), jnp.float32),
            pltpu.VMEM((ts + _HALO, D), jnp.float32),
            pltpu.VMEM((ts + _HALO, D), jnp.float32),
            pltpu.SemaphoreType.DMA((2,)),
        ],
        compiler_params=pltpu.CompilerParams(
            dimension_semantics=("arbitrary",),
            vmem_limit_bytes=100 * 1024 * 1024,
        ),
    )(x2, b1, A_wqkv, A_wo, B_w1.T, B_w2)
    return out.reshape(B, S, D)
```

```python
import functools

import jax
import jax.numpy as jnp
import jax.experimental.pallas as pl
import jax.experimental.pallas.tpu as pltpu

_H = 32
_DH = 16
_W = 8
_DIL = 2
_HALO = 16
_EPS = 1e-5


def _layernorm(x):
    m = jnp.mean(x, axis=-1, keepdims=True)
    xc = x - m
    v = jnp.mean(xc * xc, axis=-1, keepdims=True)
    return xc * jax.lax.rsqrt(v + _EPS)


def _mish(h):
    sp = jnp.log1p(jnp.exp(-jnp.abs(h))) + jnp.maximum(h, 0.0)
    return h * jnp.tanh(sp)


def _dot_t(a, b):
    return jax.lax.dot_general(a, b, (((1,), (1,)), ((), ())),
                               preferred_element_type=jnp.float32)


def _kernel(x_ref, b1_ref, wqkv_raw, wo_raw, w1_hbm, w2_hbm, o_ref,
            w1_v, w2_v, wqkv_p, wo_p, tmp, kbuf, vbuf, sems,
            *, ts, sub, d):
    i = pl.program_id(0)
    f32 = jnp.float32
    bf16 = jnp.bfloat16

    def prologue():
        cps = [
            pltpu.make_async_copy(w1_hbm, w1_v, sems.at[0]),
            pltpu.make_async_copy(w2_hbm, w2_v, sems.at[1]),
        ]
        for cp in cps:
            cp.start()
        kbuf[0, 0:_HALO, :] = jnp.zeros((_HALO, d), f32)
        vbuf[0, 0:_HALO, :] = jnp.zeros((_HALO, d), f32)

        def permute_rows(dst, base):
            for c in range(d // 128):
                for dd in range(_DH):
                    dst[base + dd * _H:base + (dd + 1) * _H, c * 128:(c + 1) * 128] = (
                        tmp[c, pl.ds(dd, _H, stride=_DH), :].astype(bf16))

        for part in range(3):
            wt = wqkv_raw[:, part * d:(part + 1) * d].astype(f32).T
            for c in range(d // 128):
                tmp[c] = wt[:, c * 128:(c + 1) * 128]
            permute_rows(wqkv_p, part * d)
        wt = wo_raw[...].astype(f32)
        for c in range(d // 128):
            tmp[c] = wt[:, c * 128:(c + 1) * 128]
        permute_rows(wo_p, 0)
        return cps

    nsub = ts // sub

    def stage_qkv(j):
        r0 = j * sub
        x = x_ref[r0:r0 + sub, :].astype(f32)
        ln1 = _layernorm(x).astype(bf16)
        qkv = _dot_t(ln1, wqkv_p[...])
        kbuf[0, _HALO + r0:_HALO + r0 + sub, :] = qkv[:, d:2 * d]
        vbuf[0, _HALO + r0:_HALO + r0 + sub, :] = qkv[:, 2 * d:3 * d]
        for sh in range(1, 4):
            for buf in (kbuf, vbuf):
                buf[sh, 8 + r0:_HALO + r0 + sub, :] = (
                    buf[0, pl.ds(8 + r0 - _DIL * sh, sub + 8), :])
        return x, qkv[:, 0:d]

    def stage_attn(j, q):
        r0 = j * sub
        pos = i * ts + r0 + jax.lax.broadcasted_iota(jnp.int32, (sub, 128), 0)
        logits = []
        for w in range(_W):
            kw = kbuf[w % 4, pl.ds(_HALO + r0 - 8 * (w // 4), sub), :]
            p = q * kw
            t = (p[:, 0:128] + p[:, 128:256]) + (p[:, 256:384] + p[:, 384:512])
            t = t + pltpu.roll(t, 32, 1)
            t = (t + pltpu.roll(t, 64, 1)) * (_DH ** -0.5)
            logits.append(jnp.where(pos >= _DIL * w, t, -1e9))
        m = logits[0]
        for w in range(1, _W):
            m = jnp.maximum(m, logits[w])
        es = [jnp.exp(l - m) for l in logits]
        den = es[0]
        for w in range(1, _W):
            den = den + es[w]
        inv = 1.0 / den
        accs = [None] * 4
        for w in range(_W):
            vw = vbuf[w % 4, pl.ds(_HALO + r0 - 8 * (w // 4), sub), :]
            for cidx in range(4):
                term = es[w] * vw[:, cidx * 128:(cidx + 1) * 128]
                accs[cidx] = term if accs[cidx] is None else accs[cidx] + term
        return jnp.concatenate([a * inv for a in accs], axis=1).astype(bf16)

    def stage_mlp(j, x, o):
        r0 = j * sub
        h = x + jnp.dot(o, wo_p[...], preferred_element_type=f32)
        ln2 = _layernorm(h).astype(bf16)
        h1 = _dot_t(ln2, w1_v[...])
        h1 = h1 + b1_ref[...].astype(f32)
        act = _mish(h1).astype(bf16)
        out = h + jnp.dot(act, w2_v[...], preferred_element_type=f32)
        o_ref[r0:r0 + sub, :] = out.astype(o_ref.dtype)

    def body(first):
        if first:
            cps = prologue()
        xs, qs = [], []
        for j in range(nsub):
            x, q = stage_qkv(j)
            xs.append(x)
            qs.append(q)
        for j in range(nsub):
            o = stage_attn(j, qs[j])
            if first and j == 0:
                cps[0].wait()
                cps[1].wait()
            stage_mlp(j, xs[j], o)

    pl.when(i == 0)(lambda: body(True))
    pl.when(i > 0)(lambda: body(False))

    kbuf[0, 0:_HALO, :] = kbuf[0, ts:ts + _HALO, :]
    vbuf[0, 0:_HALO, :] = vbuf[0, ts:ts + _HALO, :]


@jax.jit
def pallas_sequential_preLN__sliding_local_dilated__dense_activation_mish__prompt_kernel(
    A_x: jax.Array,
    A_wqkv: jax.Array,
    A_wo: jax.Array,
    B_x: jax.Array,
    B_w1: jax.Array,
    B_b1: jax.Array,
    B_w2: jax.Array,
):
    B, S, D = A_x.shape
    F = B_w1.shape[1]
    assert B == 1 and D == _H * _DH
    ts = 512
    sub = 256
    x2 = A_x.reshape(S, D)
    b1 = B_b1.reshape(1, F)
    bf16 = jnp.bfloat16

    kernel = functools.partial(_kernel, ts=ts, sub=sub, d=D)
    out = pl.pallas_call(
        kernel,
        grid=(S // ts,),
        in_specs=[
            pl.BlockSpec((ts, D), lambda i: (i, 0)),
            pl.BlockSpec((1, F), lambda i: (0, 0)),
            pl.BlockSpec((D, 3 * D), lambda i: (0, 0)),
            pl.BlockSpec((D, D), lambda i: (0, 0)),
            pl.BlockSpec(memory_space=pl.ANY),
            pl.BlockSpec(memory_space=pl.ANY),
        ],
        out_specs=pl.BlockSpec((ts, D), lambda i: (i, 0)),
        out_shape=jax.ShapeDtypeStruct((S, D), A_x.dtype),
        scratch_shapes=[
            pltpu.VMEM((F, D), bf16),
            pltpu.VMEM((F, D), bf16),
            pltpu.VMEM((3 * D, D), bf16),
            pltpu.VMEM((D, D), bf16),
            pltpu.VMEM((D // 128, D, 128), jnp.float32),
            pltpu.VMEM((4, ts + _HALO, D), jnp.float32),
            pltpu.VMEM((4, ts + _HALO, D), jnp.float32),
            pltpu.SemaphoreType.DMA((2,)),
        ],
        compiler_params=pltpu.CompilerParams(
            dimension_semantics=("arbitrary",),
            vmem_limit_bytes=100 * 1024 * 1024,
        ),
    )(x2, b1, A_wqkv, A_wo, B_w1.T, B_w2)
    return out.reshape(B, S, D)
```
